```python
import jax
import jax.numpy as jnp

def _softmax(x, axis=-1):
    return jax.nn.softmax(x, axis=axis)
def _gelu(x):
    return jax.nn.gelu(x, approximate=True)
def _silu(x):
    return jax.nn.silu(x)
def _sigmoid(x):
    return jax.nn.sigmoid(x)
def _layernorm(x, axis=-1, eps=1e-5):
    m = jnp.mean(x, axis=axis, keepdims=True)
    v = jnp.var(x, axis=axis, keepdims=True)
    return (x - m) / jnp.sqrt(v + eps)
def _scatter_add(tgt, idx, src, axis=0):
    return tgt.at[idx].add(src)
def _segment_sum(src, seg, n):
    return jax.ops.segment_sum(src, seg, n)
class _Rng:
    def __init__(self, key):
        self._k = key
    def _next(self):
        self._k, sub = jax.random.split(self._k)
        return sub
    def normal(self, shape):
        return jax.random.normal(self._next(), shape, dtype=jnp.bfloat16)
    def randint(self, lo, hi, shape):
        return jax.random.randint(self._next(), shape, lo, hi, dtype=jnp.int32)
    def uniform(self, shape, lo=0.0, hi=1.0):
        return jax.random.uniform(self._next(), shape, jnp.bfloat16, lo, hi)
    def permutation(self, n):
        return jax.random.permutation(self._next(), n)


kernel_name = 'interleave_layers__linear_attn_block__mixer_channel_mlp__prompt'

def _fwd_setup_inputs():
    _rng = _Rng(jax.random.key(int.from_bytes(__import__("os").urandom(4), "little")))
    _w = (lambda a: (lambda t: t.astype(jnp.bfloat16) if jnp.issubdtype(t.dtype, jnp.floating) else t)(jnp.asarray(a)))
    def _A_setup():
        B, S, D = 1, 2048, 576
        return {
            "x": _w((lambda *s: _rng.normal(s) * 0.05)(B, S, D)),
            "wqkv": _w((lambda *s: _rng.normal(s) * 0.05)(D, 3 * D)),
            "wo": _w((lambda *s: _rng.normal(s) * 0.05)(D, D)),
        }
    _A_in = _A_setup()

    def _B_setup():
        B, S, D, F = 1, 2048, 576, 4608
        return {
            "x": _w((lambda *s: _rng.normal(s) * 0.05)(B, S, D)),
            "w1": _w((lambda *s: _rng.normal(s) * 0.05)(D, F) * (D ** -0.5)),
            "b1": _w((lambda *s: _rng.normal(s) * 0.05)(F)),
            "w2": _w((lambda *s: _rng.normal(s) * 0.05)(F, D) * (F ** -0.5)),
            "b2": _w((lambda *s: _rng.normal(s) * 0.05)(D)),
        }
    _B_in = _B_setup()

    return {
        "A_x": _A_in["x"],
        "A_wqkv": _A_in["wqkv"],
        "A_wo": _A_in["wo"],
        "B_x": _B_in["x"],
        "B_w1": _B_in["w1"],
        "B_b1": _B_in["b1"],
        "B_w2": _B_in["w2"],
        "B_b2": _B_in["b2"],
    }

def _fwd_reference(A_x, A_wqkv, A_wo, B_x, B_w1, B_b1, B_w2, B_b2):
    def _A_ref(x, wqkv, wo):
        B, S, D = x.shape
        H = 32; Dh = D // H
        qkv = (lambda x, *d: x.transpose(*d))((x @ wqkv).reshape(B, S, 3, H, Dh), 2, 0, 3, 1, 4)
        q, k, v = qkv[0], qkv[1], qkv[2]
        phi = lambda t: jnp.where(t > 0, t + 1, jnp.exp(t)) + 1e-6
        pq, pk = phi(q), phi(k)
        kv = jnp.einsum("bhsd,bhse->bhde", pk, v)
        z = jnp.einsum("bhsd->bhd", pk)
        num = jnp.einsum("bhqd,bhde->bhqe", pq, kv)
        den = jnp.einsum("bhqd,bhd->bhq", pq, z)[..., None] + 1e-6
        o = num / den
        return (lambda x, *d: x.transpose(*d))(o, 0, 2, 1, 3).reshape(B, S, D) @ wo

    def _B_ref(x, w1, b1, w2, b2):
        y = _layernorm(x, axis=-1)
        h = _gelu(jnp.einsum("bsd,df->bsf", y, w1) + b1)
        return jnp.einsum("bsf,fd->bsd", h, w2) + b2

    x = A_x
    x = x + _A_ref(_layernorm(x, axis=-1), A_wqkv, A_wo)
    x = x + _B_ref(_layernorm(x, axis=-1), B_w1, B_b1, B_w2, B_b2)
    x = x + _A_ref(_layernorm(x, axis=-1), A_wqkv, A_wo)
    x = x + _B_ref(_layernorm(x, axis=-1), B_w1, B_b1, B_w2, B_b2)
    return x


def setup_inputs():
    _inp = _fwd_setup_inputs()
    _gk = jax.random.fold_in(jax.random.key(int.from_bytes(__import__("os").urandom(4), "little")), 2**31 - 1)
    _shapes = [[1, 2048, 576]]
    _dtypes = ['bfloat16']
    _gks = jax.random.split(_gk, len(_shapes))
    _gs = [jax.random.normal(k, s, dtype=jnp.dtype(d)) * 0.05 for k, s, d in zip(_gks, _shapes, _dtypes)]
    _inp["grad_out"] = _gs[0]
    return _inp

def reference(A_x, A_wqkv, A_wo, B_w1, B_b1, B_w2, B_b2, B_x, grad_out):
    _const = dict(B_x=B_x)
    def _f(*_d):
        return _fwd_reference(**{'A_x': _d[0], 'A_wqkv': _d[1], 'A_wo': _d[2], 'B_w1': _d[3], 'B_b1': _d[4], 'B_w2': _d[5], 'B_b2': _d[6], **_const})
    _out, _vjp = jax.vjp(_f, A_x, A_wqkv, A_wo, B_w1, B_b1, B_w2, B_b2)
    _grads = _vjp(grad_out)
    _out0 = jnp.asarray(_out)
    return (_out0, *[jnp.asarray(_g) for _g in _grads])
```

```python
import functools

import jax
import jax.numpy as jnp
from jax import lax
import jax.experimental.pallas as pl
import jax.experimental.pallas.tpu as pltpu

S, D, F, H, DH = 2048, 576, 4608, 32, 18
DE = D + 16
EPS = 1e-5
TS = 512
TF = 256
NS = S // TS
NF = F // TF
LANE = 128
BANDS = ((0, 144), (112, 272), (240, 400), (368, 528), (496, 576))
COLS = tuple((LANE * j, min(LANE * (j + 1), D)) for j in range(5))
BW = 160

F32, BF16 = jnp.float32, jnp.bfloat16
NN = (((1,), (0,)), ((), ()))
NT = (((1,), (1,)), ((), ()))
TN = (((0,), (0,)), ((), ()))
GC1 = 0.7978845608028654
GC2 = GC1 * 0.044715


def _dot(a, b, dn):
    return lax.dot_general(a, b, dn, preferred_element_type=F32)


def _ln_fwd(x):
    m = jnp.sum(x, axis=0, keepdims=True) * (1.0 / D)
    xc = x - m
    v = jnp.sum(xc * xc, axis=0, keepdims=True) * (1.0 / D) + EPS
    r = lax.rsqrt(v)
    return xc * r, m, r, v


def _ln_bwd(dy, xhat, r):
    c1 = jnp.sum(dy, axis=0, keepdims=True) * (1.0 / D)
    c2 = jnp.sum(dy * xhat, axis=0, keepdims=True) * (1.0 / D)
    return r * (dy - c1 - xhat * c2)


def _head_of(idx):
    return jnp.floor((idx.astype(F32) + 0.5) * (1.0 / DH))


def _band_mask(j):
    lo, hi = BANDS[j]
    c0, c1 = COLS[j]
    shape = (hi - lo, c1 - c0)
    r = lax.broadcasted_iota(jnp.int32, shape, 0) + lo
    c = lax.broadcasted_iota(jnp.int32, shape, 1) + c0
    return _head_of(r) == _head_of(c)


def _head_mask():
    r = lax.broadcasted_iota(jnp.int32, (H, D), 0).astype(F32)
    c = lax.broadcasted_iota(jnp.int32, (H, D), 1)
    return r == _head_of(c)


def _bcast_heads(v):
    n = v.shape[1]
    row = lax.broadcasted_iota(jnp.int32, (8, n), 0)
    pieces = []
    for g in range(H // 4):
        b = [jnp.broadcast_to(v[4 * g + i:4 * g + i + 1, :], (8, n)) for i in range(4)]
        pieces += [b[0], b[0], jnp.where(row < 2, b[0], b[1]),
                   b[1], jnp.where(row < 4, b[1], b[2]),
                   b[2], jnp.where(row < 6, b[2], b[3]), b[3], b[3]]
    return jnp.concatenate(pieces, axis=0)


def _hi_lo(x):
    hi = x.astype(BF16)
    lo = (x - hi.astype(F32)).astype(BF16)
    return hi, lo


def _lane_fold(x):
    acc = x[:, 0:LANE]
    for i in range(1, x.shape[1] // LANE):
        acc = acc + x[:, i * LANE:(i + 1) * LANE]
    return acc


def _gelu_parts(hp):
    x2 = hp * hp
    t = jnp.tanh(hp * (GC1 + GC2 * x2))
    sg = 0.5 + 0.5 * t
    return x2, t, sg


def _gelu_grad(hp, x2, t, sg):
    return sg + (0.5 * hp) * (1.0 - t * t) * (GC1 + (3.0 * GC2) * x2)


def _kernel(x_hbm, wqkv_hbm, wo_hbm, w1_hbm, b1_ref, w2_hbm, b2_ref, g_hbm,
            out_hbm, dx_hbm, dwqkv_hbm, dwo_hbm, dw1_hbm, db1_ref, dw2_hbm, db2_ref,
            xin, gin, wqkv, wo, w1e, w2, wvT,
            xT, gT, gTb, dyT, aT, pqk, rden, rows, yT, hp2, dqS,
            CT, KVT, MT, Zc, zcol, b2col, Wp, dzp, dzcol,
            dWqk, dWvT, dWo, dW1p, dW2Tp, db2a, sem):

    def tile(i):
        return pl.ds(pl.multiple_of(i * TS, TS), TS)

    def ftile(f):
        return pl.ds(pl.multiple_of(f * TF, TF), TF)

    cp_x = pltpu.make_async_copy(x_hbm.at[0], xin, sem.at[0])
    cp_wqkv = pltpu.make_async_copy(wqkv_hbm, wqkv, sem.at[1])
    cp_wo = pltpu.make_async_copy(wo_hbm, wo, sem.at[2])
    cp_w1 = pltpu.make_async_copy(w1_hbm, w1e.at[0:D, :], sem.at[3])
    cp_w2 = pltpu.make_async_copy(w2_hbm, w2, sem.at[4])
    cp_g = pltpu.make_async_copy(g_hbm.at[0], gTb, sem.at[5])
    for cp in (cp_x, cp_wqkv, cp_wo, cp_w1, cp_w2, cp_g):
        cp.start()

    row16 = lax.broadcasted_iota(jnp.int32, (16, S), 0)
    ones_rows = jnp.where(row16 == 0, 1.0, 0.0).astype(BF16)
    for l in range(2):
        aT[l, D:DE, :] = ones_rows
        yT[l, D:DE, :] = ones_rows
    rowf = lax.broadcasted_iota(jnp.int32, (16, F), 0)
    b1row = jnp.broadcast_to(b1_ref[...].reshape(1, F).astype(F32), (16, F))
    w1e[D:DE, :] = jnp.where(rowf == 0, b1row, 0.0).astype(BF16)
    b2col[...] = jnp.broadcast_to(b2_ref[...].reshape(1, D).astype(F32), (LANE, D)).T
    dWqk[...] = jnp.zeros_like(dWqk)
    dWvT[...] = jnp.zeros_like(dWvT)
    dWo[...] = jnp.zeros_like(dWo)

    cp_wqkv.wait()
    wvT[...] = wqkv[:, 2 * D:3 * D].T
    cp_x.wait()

    def a_fwd1(l):
        CT[l] = jnp.zeros((DE, D), F32)

        def body(i, carry):
            ts = tile(i)
            if l == 0:
                x = xin[:, ts].astype(F32)
                xT[:, ts] = x
            else:
                x = xT[:, ts]
            a, _, r, _ = _ln_fwd(x)
            ab = a.astype(BF16)
            aT[l, 0:D, ts] = ab
            rows[l, 0:1, ts] = r
            qk = _dot(wqkv[:, 0:2 * D], ab, TN)
            p = jnp.where(qk > 0, qk + 1.0, jnp.exp(jnp.minimum(qk, 0.0))) + 1e-6
            pb = p.astype(BF16)
            pqk[l, :, ts] = pb
            ae = jnp.concatenate([ab, aT[l, D:DE, ts]], axis=0)
            CT[l] += _dot(ae, pb[D:2 * D], NT)
            return carry

        lax.fori_loop(0, NS, body, 0)

    def a_fwd1_end(l):
        ct = CT[l]
        cth, ctl = _hi_lo(ct[0:D])
        for j in range(5):
            lo, hi = BANDS[j]
            c0, c1 = COLS[j]
            wv = wvT[lo:hi, :]
            kvt = _dot(wv, cth[:, c0:c1], NN) + _dot(wv, ctl[:, c0:c1], NN)
            kvt = jnp.where(_band_mask(j), kvt, 0.0).astype(BF16)
            KVT[l, j, 0:hi - lo, 0:c1 - c0] = kvt
            MT[l, :, c0:c1] = _dot(wo[lo:hi, :], kvt, TN).astype(BF16)
        z = ct[D:D + 1]
        Zc[...] = jnp.where(_head_mask(), jnp.broadcast_to(z, (H, D)), 0.0).astype(BF16)
        zcol[l] = jnp.broadcast_to(z, (LANE, D)).T

    def a_fwd2(l):
        def body(i, carry):
            ts = tile(i)
            pq = pqk[l, 0:D, ts]
            rd = 1.0 / (_dot(Zc[...], pq, NN) + 1e-6)
            rden[l, :, ts] = rd
            pqn = (pq.astype(F32) * _bcast_heads(rd)).astype(BF16)
            x1 = xT[:, ts] + _dot(MT[l], pqn, NN)
            u, _, r1, _ = _ln_fwd(x1)
            y, m2, r2, v2 = _ln_fwd(u)
            yT[l, 0:D, ts] = y.astype(BF16)
            rows[l, 1:2, ts] = r1
            rows[l, 2:3, ts] = r2
            rows[l, 3:4, ts] = m2
            rows[l, 4:5, ts] = v2 * r2
            xT[:, ts] = x1 + b2col[:, 0:1]
            if l == 1:
                gT[:, ts] = gTb[:, ts].astype(F32)
                dyT[:, ts] = jnp.zeros((D, TS), F32)
            return carry

        lax.fori_loop(0, NS, body, 0)

    def a_bwd1(l):
        Wp[...] = jnp.zeros_like(Wp)
        dzp[...] = jnp.zeros_like(dzp)
        ec = jnp.where(_head_mask(), 1.0, 0.0).astype(BF16)

        def body(i, carry):
            ts = tile(i)
            if l == 1:
                xin[:, ts] = xT[:, ts].astype(BF16)
                pltpu.make_async_copy(xin.at[:, ts], out_hbm.at[0, :, ts], sem.at[6]).start()
            y = yT[l, 0:D, ts].astype(F32)
            du = _ln_bwd(dyT[:, ts], y, rows[l, 2:3, ts])
            u = y * rows[l, 4:5, ts] + rows[l, 3:4, ts]
            dx = gT[:, ts] + _ln_bwd(du, u, rows[l, 1:2, ts])
            gT[:, ts] = dx
            dxb = dx.astype(BF16)
            pq = pqk[l, 0:D, ts].astype(F32)
            rd = rden[l, :, ts]
            rb = _bcast_heads(rd)
            pqn = pq * rb
            dpqn = _dot(MT[l], dxb, TN)
            Wp[...] += _dot(pqn.astype(BF16), dxb, NT)
            t = (dpqn * pqn).astype(BF16)
            dden = -(rd * _dot(ec, t, NN))
            db = _bcast_heads(dden)
            dpq = dpqn * rb + zcol[l, :, 0:1] * db
            dqS[:, ts] = (dpq * jnp.minimum(pq - 1e-6, 1.0)).astype(BF16)
            dzp[...] += _lane_fold(pq * db)
            return carry

        lax.fori_loop(0, NS, body, 0)

    def a_bwd1_end(l):
        wh, wl = _hi_lo(Wp[...])
        cth, ctl = _hi_lo(CT[l, 0:D, :])
        for j in range(5):
            lo, hi = BANDS[j]
            c0, c1 = COLS[j]
            kvt = KVT[l, j, 0:hi - lo, 0:c1 - c0]
            dWo[lo:hi, :] += _dot(kvt, wh[c0:c1], NN) + _dot(kvt, wl[c0:c1], NN)
            wob = wo[lo:hi, :]
            dkvt = _dot(wob, wh[c0:c1], NT) + _dot(wob, wl[c0:c1], NT)
            dkvt = jnp.where(_band_mask(j), dkvt, 0.0).astype(BF16)
            wqkv[:, 2 * D + c0:2 * D + c1] = _dot(wvT[lo:hi, :], dkvt, TN).astype(BF16)
            dWvT[lo:hi, :] += _dot(dkvt, cth[:, c0:c1], NT) + _dot(dkvt, ctl[:, c0:c1], NT)
        dzcol[...] = jnp.broadcast_to(jnp.sum(dzp[...], axis=1, keepdims=True), (D, LANE))

    def a_bwd2(l):
        def body(i, carry):
            ts = tile(i)
            ab = aT[l, 0:D, ts]
            pkb = pqk[l, D:2 * D, ts]
            dpk = _dot(wqkv[:, 2 * D:3 * D], ab, TN) + dzcol[:, 0:1]
            dkb = (dpk * jnp.minimum(pkb.astype(F32) - 1e-6, 1.0)).astype(BF16)
            dqk = jnp.concatenate([dqS[:, ts], dkb], axis=0)
            dWqk[...] += _dot(ab, dqk, NT)
            da = _dot(wqkv[...], jnp.concatenate([dqk, pkb], axis=0), NN)
            dx = gT[:, ts] + _ln_bwd(da, ab.astype(F32), rows[l, 0:1, ts])
            if l == 1:
                gT[:, ts] = dx
                gTb[:, ts] = dx.astype(BF16)
                dyT[:, ts] = jnp.zeros((D, TS), F32)
            else:
                gin[:, ts] = dx.astype(BF16)
                pltpu.make_async_copy(gin.at[:, ts], dx_hbm.at[0, :, ts], sem.at[7]).start()
            return carry

        lax.fori_loop(0, NS, body, 0)

    def b_fwd():
        def body(f, carry):
            fs = ftile(f)
            hp = _dot(w1e[:, fs], yT[0], TN)
            hp2[fs, :] = hp.astype(BF16)
            _, _, sg = _gelu_parts(hp)
            h = (hp * sg).astype(BF16)
            xT[...] += _dot(w2[:, fs], h, NN)
            return carry

        lax.fori_loop(0, NF, body, 0)

    def b_fwd_bwd():
        db2a[...] = _dot(yT[1, D:DE, :], gTb[...], NT)

        def body(f, carry):
            fs = ftile(f)
            w1t = w1e[:, fs]
            w2t = w2[:, fs]
            ye = yT[1]
            g = gTb[...]
            hp = _dot(w1t, ye, TN)
            dh = _dot(w2t, g, TN)
            x2, t, sg = _gelu_parts(hp)
            h = (hp * sg).astype(BF16)
            dhp = (dh * _gelu_grad(hp, x2, t, sg)).astype(BF16)
            xT[...] += _dot(w2t, h, NN)
            dyT[...] += _dot(w1t[0:D], dhp, NN)
            dW1p[:, fs] = _dot(ye, dhp, NT).astype(dW1p.dtype)
            dW2Tp[:, fs] = _dot(g, h, NT).astype(dW2Tp.dtype)
            return carry

        lax.fori_loop(0, NF, body, 0)

    def b_bwd():
        db2a[...] += _dot(yT[0, D:DE, :], gTb[...], NT)
        db2_ref[...] = db2a[0:1, :].reshape(D).astype(BF16)

        def body(f, carry):
            fs = ftile(f)
            w1t = w1e[0:D, fs]
            w2t = w2[:, fs]
            ye = yT[0]
            g = gTb[...]
            hp = hp2[fs, :].astype(F32)
            dh = _dot(w2t, g, TN)
            x2, t, sg = _gelu_parts(hp)
            h = (hp * sg).astype(BF16)
            dhp = (dh * _gelu_grad(hp, x2, t, sg)).astype(BF16)
            dyT[...] += _dot(w1t, dhp, NN)
            dw1 = dW1p[:, fs].astype(F32) + _dot(ye, dhp, NT)
            dw2t = dW2Tp[:, fs].astype(F32) + _dot(g, h, NT)
            w1e[:, fs] = dw1.astype(BF16)
            w2[:, fs] = dw2t.astype(BF16)
            pltpu.make_async_copy(w1e.at[0:D, fs], dw1_hbm.at[:, fs], sem.at[8]).start()
            pltpu.make_async_copy(w2.at[:, fs], dw2_hbm.at[:, fs], sem.at[9]).start()
            return carry

        lax.fori_loop(0, NF, body, 0)
        db1_ref[...] = w1e[D:DE, :].astype(F32)[0:1, :].reshape(F).astype(BF16)

    with jax.named_scope("a_fwd1_0"):
        a_fwd1(0)
    cp_wo.wait()
    with jax.named_scope("a_fwd1e_0"):
        a_fwd1_end(0)
    with jax.named_scope("a_fwd2_0"):
        a_fwd2(0)
    cp_w1.wait()
    cp_w2.wait()
    with jax.named_scope("b_fwd"):
        b_fwd()
    with jax.named_scope("a_fwd1_1"):
        a_fwd1(1)
    with jax.named_scope("a_fwd1e_1"):
        a_fwd1_end(1)
    cp_g.wait()
    with jax.named_scope("a_fwd2_1"):
        a_fwd2(1)
    with jax.named_scope("b_fwd_bwd"):
        b_fwd_bwd()
    with jax.named_scope("a_bwd1_1"):
        a_bwd1(1)
    with jax.named_scope("a_bwd1e_1"):
        a_bwd1_end(1)
    with jax.named_scope("a_bwd2_1"):
        a_bwd2(1)
    with jax.named_scope("b_bwd"):
        b_bwd()
    with jax.named_scope("a_bwd1_0"):
        a_bwd1(0)
    with jax.named_scope("a_bwd1e_0"):
        a_bwd1_end(0)
        wo[...] = dWo[...].astype(BF16)
        cp_dwo = pltpu.make_async_copy(wo, dwo_hbm, sem.at[10])
        cp_dwo.start()
    with jax.named_scope("a_bwd2_0"):
        a_bwd2(0)
    with jax.named_scope("final"):
        wqkv[:, 0:2 * D] = dWqk[...].astype(BF16)
        wqkv[:, 2 * D:3 * D] = dWvT[...].T.astype(BF16)
        cp_dwqkv = pltpu.make_async_copy(wqkv, dwqkv_hbm, sem.at[11])
        cp_dwqkv.start()
        pltpu.make_async_copy(xin, out_hbm.at[0], sem.at[6]).wait()
        pltpu.make_async_copy(w1e.at[0:D, :], dw1_hbm, sem.at[8]).wait()
        pltpu.make_async_copy(w2, dw2_hbm, sem.at[9]).wait()
        cp_dwo.wait()
        pltpu.make_async_copy(gin, dx_hbm.at[0], sem.at[7]).wait()
        cp_dwqkv.wait()


@jax.jit
def pallas_interleave_layers__linear_attn_block__mixer_channel_mlp__prompt_kernel(
    A_x: jax.Array,
    A_wqkv: jax.Array,
    A_wo: jax.Array,
    B_x: jax.Array,
    B_w1: jax.Array,
    B_b1: jax.Array,
    B_w2: jax.Array,
    B_b2: jax.Array,
    grad_out: jax.Array,
):
    del B_x
    hbm = pl.BlockSpec(memory_space=pl.ANY)
    vmem = pl.BlockSpec(memory_space=pltpu.VMEM)
    sds = jax.ShapeDtypeStruct
    out_shape = (
        sds((1, D, S), BF16), sds((1, D, S), BF16), sds((D, 3 * D), BF16), sds((D, D), BF16),
        sds((D, F), BF16), sds((F,), BF16), sds((D, F), BF16), sds((D,), BF16),
    )
    V = pltpu.VMEM
    scratch = [
        V((D, S), BF16), V((D, S), BF16),
        V((D, 3 * D), BF16), V((D, D), BF16),
        V((DE, F), BF16), V((D, F), BF16), V((D, D), BF16),
        V((D, S), F32), V((D, S), F32), V((D, S), BF16), V((D, S), F32),
        V((2, DE, S), BF16), V((2, 2 * D, S), BF16),
        V((2, H, S), F32), V((2, 8, S), F32),
        V((2, DE, S), BF16), V((F, S), BF16), V((D, S), BF16),
        V((2, DE, D), F32), V((2, 5, BW, LANE), BF16), V((2, D, D), BF16),
        V((H, D), BF16), V((2, D, LANE), F32), V((D, LANE), F32),
        V((D, D), F32), V((D, LANE), F32), V((D, LANE), F32),
        V((D, 2 * D), F32), V((D, D), F32), V((D, D), F32),
        V((DE, F), F32), V((D, F), F32), V((16, D), F32),
        pltpu.SemaphoreType.DMA((12,)),
    ]
    outT, dxT, dwqkv, dwo, dw1, db1, dw2T, db2 = pl.pallas_call(
        _kernel,
        out_shape=out_shape,
        in_specs=[hbm, hbm, hbm, hbm, vmem, hbm, vmem, hbm],
        out_specs=(hbm, hbm, hbm, hbm, hbm, vmem, hbm, vmem),
        scratch_shapes=scratch,
        compiler_params=pltpu.CompilerParams(vmem_limit_bytes=126 * 1024 * 1024),
    )(jnp.swapaxes(A_x, 1, 2), A_wqkv, A_wo, B_w1, B_b1, B_w2.T, B_b2,
      jnp.swapaxes(grad_out, 1, 2))
    return (jnp.swapaxes(outT, 1, 2), jnp.swapaxes(dxT, 1, 2), dwqkv, dwo, dw1, db1,
            dw2T.T, db2)
```
